```python
import jax
import jax.numpy as jnp

def _softmax(x, axis=-1):
    return jax.nn.softmax(x, axis=axis)
def _gelu(x):
    return jax.nn.gelu(x, approximate=True)
def _silu(x):
    return jax.nn.silu(x)
def _sigmoid(x):
    return jax.nn.sigmoid(x)
def _layernorm(x, axis=-1, eps=1e-5):
    m = jnp.mean(x, axis=axis, keepdims=True)
    v = jnp.var(x, axis=axis, keepdims=True)
    return (x - m) / jnp.sqrt(v + eps)
def _scatter_add(tgt, idx, src, axis=0):
    return tgt.at[idx].add(src)
def _segment_sum(src, seg, n):
    return jax.ops.segment_sum(src, seg, n)
class _Rng:
    def __init__(self, key):
        self._k = key
    def _next(self):
        self._k, sub = jax.random.split(self._k)
        return sub
    def normal(self, shape):
        return jax.random.normal(self._next(), shape, dtype=jnp.bfloat16)
    def randint(self, lo, hi, shape):
        return jax.random.randint(self._next(), shape, lo, hi, dtype=jnp.int32)
    def uniform(self, shape, lo=0.0, hi=1.0):
        return jax.random.uniform(self._next(), shape, jnp.bfloat16, lo, hi)
    def permutation(self, n):
        return jax.random.permutation(self._next(), n)


kernel_name = 'standalone__batchnorm__sampling'

def setup_inputs():
    _rng = _Rng(jax.random.key(int.from_bytes(__import__("os").urandom(4), "little")))
    _w = (lambda a: (lambda t: t.astype(jnp.bfloat16) if jnp.issubdtype(t.dtype, jnp.floating) else t)(jnp.asarray(a)))
    B, S, C = 1024, 32, 576
    K = 3
    return {
        "x": _w((lambda *s: _rng.normal(s) * 0.05)(B, S, C)),
        "w": _w((lambda *s: _rng.normal(s) * 0.05)(K, C, C) * (1.0 / (K * C) ** 0.5)),
        "mean": _w((lambda *s: _rng.normal(s) * 0.05)(C) * 0.1),
        "var": _w(jnp.abs((lambda *s: _rng.normal(s) * 0.05)(C)) + 0.5),
        "g": _w((lambda *s: _rng.normal(s) * 0.05)(C) + 1.0),
        "b": _w((lambda *s: _rng.normal(s) * 0.05)(C) * 0.1),
    }

def reference(x, w, mean, var, g, b):
    K = 3
    P = K // 2
    S = x.shape[1]
    xp = jnp.pad(x, ((0, 0), (P, P), (0, 0)))
    y = sum(jnp.einsum('bsc,cd->bsd', xp[:, k:k + S, :], w[k]) for k in range(K))
    inv_std = 1.0 / jnp.sqrt(var + 1e-5)
    y = (y - mean) * (g * inv_std) + b
    return _silu(y)
```

```python
import numpy as np
import jax
import jax.numpy as jnp
from jax import lax
import jax.experimental.pallas as pl
import jax.experimental.pallas.tpu as pltpu

_F = np.float32
_PA, _PB = 2.0 / 3.0, 1.5
_LANES = 128


def _toom_cook_4_3(a, b):
    pts = [0.0, a, -a, b, -b]

    def vander(k):
        m = np.zeros((6, k))
        for j, p in enumerate(pts):
            m[j] = [p ** e for e in range(k)]
        m[5, k - 1] = 1.0
        return m

    at, g, bt = vander(4).T, vander(3), np.linalg.inv(vander(6)).T
    sc = np.array([bt[j, 4] for j in range(5)] + [bt[5, 5]])
    return at, g * sc[:, None], bt / sc[:, None]


@jax.jit
def pallas_standalone__batchnorm__sampling_kernel(
    x: jax.Array,
    w: jax.Array,
    mean: jax.Array,
    var: jax.Array,
    g: jax.Array,
    b: jax.Array,
):
    B, S, C = x.shape
    nb = _LANES
    assert S % 4 == 0 and B % nb == 0 and C % 16 == 0 and w.shape[0] == 3
    NT = S // 4
    NBT = B // nb
    KT = pl.cdiv(C, 128)
    f32, bf16 = jnp.float32, jnp.bfloat16
    _, G, _ = _toom_cook_4_3(_PA, _PB)
    pa, pb = _PA, _PB
    a2, b2 = pa * pa, pb * pb

    def kernel(x_hbm, w_hbm, mean_ref, var_ref, g_ref, b_ref, o_hbm,
               xbuf, obuf, wbuf, gt_ref, sh_ref, xsem, osem, wsem):
        def xcopy(bt, slot):
            return pltpu.make_async_copy(
                x_hbm.at[:, :, pl.ds(bt * nb, nb)], xbuf.at[slot], xsem.at[slot])

        def ocopy(bt, slot, i):
            return pltpu.make_async_copy(
                obuf.at[slot, pl.ds(4 * i, 4)],
                o_hbm.at[pl.ds(4 * i, 4), :, pl.ds(bt * nb, nb)], osem.at[slot])

        wcopy = pltpu.make_async_copy(w_hbm, wbuf, wsem)
        wcopy.start()
        xcopy(0, 0).start()

        row = lambda r: r[...].astype(f32).reshape(1, C)
        scale = row(g_ref) * (1.0 / jnp.sqrt(row(var_ref) + 1e-5))
        shift = row(b_ref) - row(mean_ref) * scale
        scale = scale * _F(0.5)
        shift = shift * _F(0.5)
        sh_ref[...] = jnp.broadcast_to(shift, (128, C)).T
        wcopy.wait()
        for kt in range(KT):
            lo = kt * 128
            hi = min(lo + 128, C)
            w0, w1, w2 = (wbuf[k, lo:hi].astype(f32) for k in range(3))

            def put(j, v, lo=lo, hi=hi, kt=kt):
                if hi - lo < 128:
                    v = jnp.concatenate([v, jnp.zeros((128 - (hi - lo), C), f32)], axis=0)
                gt_ref[j, kt] = pltpu.bitcast(v.T.astype(bf16), jnp.int32)

            put(0, w0 * (scale * _F(G[0, 0])))
            put(5, w2 * (scale * _F(G[5, 2])))
            for j in (1, 3):
                ev = w0 * (scale * _F(G[j, 0])) + w2 * (scale * _F(G[j, 2]))
                od = w1 * (scale * _F(G[j, 1]))
                put(j, ev + od)
                put(j + 1, ev - od)

        def body(bt, carry):
            slot = bt % 2

            @pl.when(bt + 1 < NBT)
            def _():
                xcopy(bt + 1, 1 - slot).start()

            @pl.when(bt >= 2)
            def _():
                for i in range(NT):
                    ocopy(bt - 2, slot, i).wait()

            xcopy(bt, slot).wait()
            for i in range(NT):
                d = [xbuf[slot, s].astype(f32) if 0 <= s < S else None
                     for s in range(4 * i - 1, 4 * i + 5)]
                t0 = d[4] - _F(a2 + b2) * d[2]
                if d[0] is not None:
                    t0 = t0 + d[0]
                t5 = d[1] - _F(a2 + b2) * d[3]
                if d[5] is not None:
                    t5 = t5 + d[5]
                u1 = d[4] - _F(b2) * d[2]
                v1 = _F(pa) * d[3] - _F(pb) * d[1]
                u2 = d[4] - _F(a2) * d[2]
                v2 = _F(pb) * d[3] - _F(pa) * d[1]
                ts = [t.astype(bf16) for t in (t0, u1 + v1, u1 - v1, u2 + v2, u2 - v2, t5)]

                def dot(j):
                    acc = None
                    for kt in range(KT):
                        lo = kt * 128
                        hi = min(lo + 128, C)
                        gt = pltpu.bitcast(gt_ref[j, kt], bf16)
                        p = jnp.dot(gt[:, 0:hi - lo], ts[j][lo:hi], preferred_element_type=f32)
                        acc = p if acc is None else acc + p
                    return acc

                m = [dot(j) for j in range(6)]
                sh = sh_ref[...]
                s12 = m[1] + m[2]
                d12 = m[1] - m[2]
                s34 = m[3] + m[4]
                d34 = m[3] - m[4]
                y0 = (m[0] + sh) + (s12 + s34)
                y1 = (_F(pa) * d12 + _F(pb) * d34) + sh
                y2 = (_F(a2) * s12 + _F(b2) * s34) + sh
                y3 = (_F(a2 * pa) * d12 + _F(b2 * pb) * d34) + (m[5] + sh)
                for t, h in enumerate((y0, y1, y2, y3)):
                    obuf[slot, 4 * i + t] = (h + h * jnp.tanh(h)).astype(obuf.dtype)
                ocopy(bt, slot, i).start()
            return carry

        lax.fori_loop(0, NBT, body, 0)
        for bt in range(max(NBT - 2, 0), NBT):
            for i in range(NT):
                ocopy(bt, bt % 2, i).wait()

    x_t = jnp.transpose(x, (1, 2, 0))
    vmem = pl.BlockSpec(memory_space=pltpu.VMEM)
    hbm = pl.BlockSpec(memory_space=pl.ANY)
    out_t = pl.pallas_call(
        kernel,
        in_specs=[hbm, hbm, vmem, vmem, vmem, vmem],
        out_specs=hbm,
        out_shape=jax.ShapeDtypeStruct((S, C, B), x.dtype),
        scratch_shapes=[
            pltpu.VMEM((2, S, C, nb), x.dtype),
            pltpu.VMEM((2, S, C, nb), x.dtype),
            pltpu.VMEM((3, C, C), w.dtype),
            pltpu.VMEM((6, KT, C // 2, 128), jnp.int32),
            pltpu.VMEM((C, 128), f32),
            pltpu.SemaphoreType.DMA((2,)),
            pltpu.SemaphoreType.DMA((2,)),
            pltpu.SemaphoreType.DMA(()),
        ],
        compiler_params=pltpu.CompilerParams(vmem_limit_bytes=64 * 1024 * 1024),
    )(x_t, w, mean, var, g, b)
    return jnp.transpose(out_t, (2, 0, 1))
```

```python
import numpy as np
import jax
import jax.numpy as jnp
from jax import lax
import jax.experimental.pallas as pl
import jax.experimental.pallas.tpu as pltpu

_F = np.float32
_POINTS = {4: (2.0 / 3.0, 1.5), 6: (1.0, 0.5, 2.0)}
_NB = 128


def _toom_cook(m):
    n = m + 2
    pts = [0.0]
    for p in _POINTS[m]:
        pts += [p, -p]

    def vander(k):
        mat = np.zeros((n, k))
        for j, p in enumerate(pts):
            mat[j] = [p ** e for e in range(k)]
        mat[n - 1, k - 1] = 1.0
        return mat

    at, g, bt = vander(m).T, vander(3), np.linalg.inv(vander(n)).T
    sc = np.array([bt[j, n - 2] for j in range(n - 1)] + [bt[n - 1, n - 1]])
    bt, g = bt / sc[:, None], g * sc[:, None]
    bt[np.abs(bt) < 1e-9] = 0.0
    g[np.abs(g) < 1e-12] = 0.0
    return at, g, bt


def _lin(terms):
    groups = {}
    for c, v in terms:
        if v is not None and abs(c) > 1e-9:
            groups.setdefault(round(abs(float(c)), 9), []).append((1.0 if c > 0 else -1.0, v))
    acc = None
    for k in sorted(groups, key=lambda k: (k != 1.0, k)):
        grp = sorted(groups[k], key=lambda t: -t[0])
        s0, v = grp[0]
        for s, vv in grp[1:]:
            v = v + vv if s == s0 else v - vv
        if k == 1.0:
            acc = v if s0 > 0 else -v
        else:
            acc = _F(k * s0) * v if acc is None else acc + _F(k * s0) * v
    return acc


def _tiling(S):
    n6 = (S - 8) // 6 if S >= 8 else 0
    while (S - 6 * n6) % 4:
        n6 -= 1
    assert n6 >= 0
    return (6,) * n6 + (4,) * ((S - 6 * n6) // 4)


@jax.jit
def pallas_standalone__batchnorm__sampling_kernel(
    x: jax.Array,
    w: jax.Array,
    mean: jax.Array,
    var: jax.Array,
    g: jax.Array,
    b: jax.Array,
):
    B, S, C = x.shape
    nb = _NB
    assert B % nb == 0 and B // nb >= 2 and C % 16 == 0 and w.shape[0] == 3
    tiles = _tiling(S)
    starts = [sum(tiles[:i]) for i in range(len(tiles))]
    sizes = sorted(set(tiles), reverse=True)
    tc = {m: _toom_cook(m) for m in sizes}
    goff, ng = {}, 0
    for m in sizes:
        goff[m] = ng
        ng += m + 2
    NBT = B // nb
    KT = pl.cdiv(C, 128)
    f32, bf16 = jnp.float32, jnp.bfloat16

    def kernel(x_hbm, w_hbm, mean_ref, var_ref, g_ref, b_ref, o_hbm,
               xbuf, obuf, wbuf, gt_ref, sh_ref, xsem, osem, wsem):
        def xcopy(bt, slot):
            return pltpu.make_async_copy(
                x_hbm.at[:, :, pl.ds(bt * nb, nb)], xbuf.at[slot], xsem.at[slot])

        def ocopy(bt, slot, i):
            return pltpu.make_async_copy(
                obuf.at[slot, pl.ds(starts[i], tiles[i])],
                o_hbm.at[pl.ds(starts[i], tiles[i]), :, pl.ds(bt * nb, nb)], osem.at[slot])

        wcopy = pltpu.make_async_copy(w_hbm, wbuf, wsem)
        wcopy.start()
        xcopy(0, 0).start()

        row = lambda r: r[...].astype(f32).reshape(1, C)
        scale = row(g_ref) * (1.0 / jnp.sqrt(row(var_ref) + 1e-5))
        shift = row(b_ref) - row(mean_ref) * scale
        scale = scale * _F(0.5)
        shift = shift * _F(0.5)
        sh_ref[...] = jnp.broadcast_to(shift, (128, C)).T
        wcopy.wait()
        for kt in range(KT):
            lo = kt * 128
            hi = min(lo + 128, C)
            w0, w1, w2 = (wbuf[k, lo:hi].astype(f32) for k in range(3))

            def put(j, v, lo=lo, hi=hi, kt=kt):
                if hi - lo < 128:
                    v = jnp.concatenate([v, jnp.zeros((128 - (hi - lo), C), f32)], axis=0)
                gt_ref[j, kt] = pltpu.bitcast(v.T.astype(bf16), jnp.int32)

            for m in sizes:
                G, o, n = tc[m][1], goff[m], m + 2
                put(o, w0 * (scale * _F(G[0, 0])))
                put(o + n - 1, w2 * (scale * _F(G[n - 1, 2])))
                for j in range(1, n - 1, 2):
                    ev = w0 * (scale * _F(G[j, 0])) + w2 * (scale * _F(G[j, 2]))
                    od = w1 * (scale * _F(G[j, 1]))
                    put(o + j, ev + od)
                    put(o + j + 1, ev - od)

        def body(bt, carry):
            slot = bt % 2
            xcopy(bt, slot).wait()

            @pl.when(bt + 1 < NBT)
            def _():
                xcopy(bt + 1, 1 - slot).start()

            @pl.when(bt >= 2)
            def _():
                for i in range(len(tiles)):
                    ocopy(bt - 2, slot, i).wait()

            for i, m in enumerate(tiles):
                AT, _, BT = tc[m]
                n, s0 = m + 2, starts[i]
                d = [xbuf[slot, s].astype(f32) if 0 <= s < S else None
                     for s in range(s0 - 1, s0 + m + 1)]
                ts = [None] * n
                ts[0] = _lin([(BT[0, t], d[t]) for t in range(n)])
                ts[n - 1] = _lin([(BT[n - 1, t], d[t]) for t in range(n)])
                for j in range(1, n - 1, 2):
                    ev = _lin([(BT[j, t], d[t]) for t in range(0, n, 2)])
                    od = _lin([(BT[j, t], d[t]) for t in range(1, n, 2)])
                    ts[j], ts[j + 1] = ev + od, ev - od
                ts = [t.astype(bf16) for t in ts]

                def dot(j):
                    acc = None
                    for kt in range(KT):
                        lo = kt * 128
                        hi = min(lo + 128, C)
                        gt = pltpu.bitcast(gt_ref[goff[m] + j, kt], bf16)
                        p = jnp.dot(gt[:, 0:hi - lo], ts[j][lo:hi], preferred_element_type=f32)
                        acc = p if acc is None else acc + p
                    return acc

                mm = [dot(j) for j in range(n)]
                sh = sh_ref[...]
                fold = _POINTS[m][0] == 1.0
                if fold:
                    mm[1] = mm[1] + sh
                sd = {j: (mm[j] + mm[j + 1], mm[j] - mm[j + 1]) for j in range(1, n - 1, 2)}
                for o in range(m):
                    terms = [(AT[o, j], sd[j][o % 2]) for j in range(1, n - 1, 2)]
                    terms += [(AT[o, 0], mm[0]), (AT[o, n - 1], mm[n - 1])]
                    h = _lin(terms)
                    if not fold:
                        h = h + sh
                    obuf[slot, s0 + o] = (h + h * jnp.tanh(h)).astype(obuf.dtype)
                ocopy(bt, slot, i).start()
            return carry

        lax.fori_loop(0, NBT, body, 0)
        for bt in range(NBT - 2, NBT):
            for i in range(len(tiles)):
                ocopy(bt, bt % 2, i).wait()

    x_t = jnp.transpose(x, (1, 2, 0))
    vmem = pl.BlockSpec(memory_space=pltpu.VMEM)
    hbm = pl.BlockSpec(memory_space=pl.ANY)
    out_t = pl.pallas_call(
        kernel,
        in_specs=[hbm, hbm, vmem, vmem, vmem, vmem],
        out_specs=hbm,
        out_shape=jax.ShapeDtypeStruct((S, C, B), x.dtype),
        scratch_shapes=[
            pltpu.VMEM((2, S, C, nb), x.dtype),
            pltpu.VMEM((2, S, C, nb), x.dtype),
            pltpu.VMEM((3, C, C), w.dtype),
            pltpu.VMEM((ng, KT, C // 2, 128), jnp.int32),
            pltpu.VMEM((C, 128), f32),
            pltpu.SemaphoreType.DMA((2,)),
            pltpu.SemaphoreType.DMA((2,)),
            pltpu.SemaphoreType.DMA(()),
        ],
        compiler_params=pltpu.CompilerParams(vmem_limit_bytes=100 * 1024 * 1024),
    )(x_t, w, mean, var, g, b)
    return jnp.transpose(out_t, (2, 0, 1))
```
